```python
import os as _os
_os.environ.setdefault("JAX_PLATFORMS", "cpu")
import jax
import jax.numpy as jnp

def _softmax(x, axis=-1):
    return jax.nn.softmax(x, axis=axis)
def _gelu(x):
    return jax.nn.gelu(x, approximate=True)
def _silu(x):
    return jax.nn.silu(x)
def _sigmoid(x):
    return jax.nn.sigmoid(x)
def _layernorm(x, axis=-1, eps=1e-5):
    m = jnp.mean(x, axis=axis, keepdims=True)
    v = jnp.var(x, axis=axis, keepdims=True)
    return (x - m) / jnp.sqrt(v + eps)
def _scatter_add(tgt, idx, src, axis=0):
    return tgt.at[idx].add(src)
def _segment_sum(src, seg, n):
    return jax.ops.segment_sum(src, seg, n)
class _Rng:
    def __init__(self, key):
        self._k = key
    def _next(self):
        self._k, sub = jax.random.split(self._k)
        return sub
    def normal(self, shape):
        return jax.random.normal(self._next(), shape, dtype=jnp.bfloat16)
    def randint(self, lo, hi, shape):
        return jax.random.randint(self._next(), shape, lo, hi, dtype=jnp.int32)
    def uniform(self, shape, lo=0.0, hi=1.0):
        return jax.random.uniform(self._next(), shape, jnp.bfloat16, lo, hi)
    def permutation(self, n):
        return jax.random.permutation(self._next(), n)


kernel_name = 'parallel_sum__ssm_conv_s5__geglu_ffn__prompt'

def setup_inputs():
    _rng = _Rng(jax.random.key(int.from_bytes(__import__("os").urandom(4), "little")))
    _w = (lambda a: (lambda t: t.astype(jnp.bfloat16) if jnp.issubdtype(t.dtype, jnp.floating) else t)(jnp.asarray(a)))
    def _A_setup():
        B, S, D = 1, 2048, 512
        P = D
        Lambda_re = -0.5 * jnp.exp((lambda *s: _rng.normal(s) * 0.8)(P))
        Lambda_im = (lambda *s: _rng.normal(s) * 0.8)(P) * 1.0
        B_re = (lambda *s: _rng.normal(s) * 0.8)(P, D) * (D ** -0.5)
        B_im = (lambda *s: _rng.normal(s) * 0.8)(P, D) * (D ** -0.5)
        C_re = (lambda *s: _rng.normal(s) * 0.8)(D, P) * (P ** -0.5)
        C_im = (lambda *s: _rng.normal(s) * 0.8)(D, P) * (P ** -0.5)
        log_dt = (lambda *s: _rng.normal(s) * 0.8)(P) * 0.3 - 2.0
        Dskip = (lambda *s: _rng.normal(s) * 0.8)(D)
        return {
            "x": _w((lambda *s: _rng.normal(s) * 0.05)(B, S, D)),
            "Lambda_re": _w(Lambda_re),
            "Lambda_im": _w(Lambda_im),
            "B_re": _w(B_re),
            "B_im": _w(B_im),
            "C_re": _w(C_re),
            "C_im": _w(C_im),
            "log_dt": _w(log_dt),
            "Dskip": _w(Dskip),
        }
    _A_in = _A_setup()

    def _B_setup():
        B, S, D, F = 1, 2048, 512, 1376
        return {
            "x": _w((lambda *s: _rng.normal(s) * 0.05)(B, S, D)),
            "w_gate": _w((lambda *s: _rng.normal(s) * 0.05)(D, F)),
            "w_up": _w((lambda *s: _rng.normal(s) * 0.05)(D, F)),
            "w_down": _w((lambda *s: _rng.normal(s) * 0.05)(F, D)),
        }
    _B_in = _B_setup()

    return {
        "A_x": _A_in["x"],
        "A_Lambda_re": _A_in["Lambda_re"],
        "A_Lambda_im": _A_in["Lambda_im"],
        "A_B_re": _A_in["B_re"],
        "A_B_im": _A_in["B_im"],
        "A_C_re": _A_in["C_re"],
        "A_C_im": _A_in["C_im"],
        "A_log_dt": _A_in["log_dt"],
        "A_Dskip": _A_in["Dskip"],
        "B_x": _B_in["x"],
        "B_w_gate": _B_in["w_gate"],
        "B_w_up": _B_in["w_up"],
        "B_w_down": _B_in["w_down"],
    }

def reference(A_x, A_Lambda_re, A_Lambda_im, A_B_re, A_B_im, A_C_re, A_C_im, A_log_dt, A_Dskip, B_x, B_w_gate, B_w_up, B_w_down):
    def _A_ref(x, Lambda_re, Lambda_im, B_re, B_im, C_re, C_im, log_dt, Dskip):
        Bsz, L, H = x.shape
        Lam = Lambda_re + 1j * Lambda_im
        Bmat = B_re + 1j * B_im
        Cmat = C_re + 1j * C_im
        dt = jnp.exp(log_dt)
        Lam_bar = jnp.exp(dt * Lam)
        B_bar = ((Lam_bar - 1.0) / Lam)[:, None] * Bmat
        Bu = jnp.einsum("bld,pd->blp", x + 0j, B_bar)
        h = jnp.zeros_like(Bu[:, 0, :])
        hs = []
        for t in range(L):
            h = Lam_bar[None, :] * h + Bu[:, t, :]
            hs.append(h)
        hseq = jnp.stack(hs, 1)
        y = 2.0 * jnp.einsum("blp,dp->bld", hseq, Cmat).real + x * Dskip[None, None, :]
        return y

    def _B_ref(x, w_gate, w_up, w_down):
        return (_gelu(x @ w_gate) * (x @ w_up)) @ w_down

    x = A_x
    xn = _layernorm(x, axis=-1)
    return x + _A_ref(xn, A_Lambda_re, A_Lambda_im, A_B_re, A_B_im, A_C_re, A_C_im, A_log_dt, A_Dskip) + _B_ref(xn, B_w_gate, B_w_up, B_w_down)
```

```python
import functools
import math
import jax
import jax.numpy as jnp
from jax import lax
import jax.experimental.pallas as pl
import jax.experimental.pallas.tpu as pltpu

_NT = (((1,), (1,)), ((), ()))


def _gelu_tanh(x):
    c = math.sqrt(2.0 / math.pi)
    return 0.5 * x * (1.0 + jnp.tanh(c * (x + 0.044715 * (x * x * x))))


def _make_kernel(TL, D, P, F, UNROLL):
    CH = TL // 8
    PITCH = CH + 8
    NC = P // 128
    ND = D // 128

    def kernel(x_ref, lre_ref, lim_ref, ldt_ref, dsk_ref, bre_hbm, bim_hbm, cre_hbm, cim_hbm,
               wg_hbm, wu_hbm, wd_hbm, o_ref,
               bre_ref, bim_ref, cre_ref, cim_ref, wg_ref, wu_ref, wd_ref, sems,
               par_ref, pwr_ref, pwi_ref, car_ref, xs_ref, xp_ref, bur_ref, bui_ref, hcat_ref, ys_ref):
        step = pl.program_id(0)

        copies = [pltpu.make_async_copy(h, v, sems.at[k]) for k, (h, v) in enumerate(
            [(bre_hbm, bre_ref), (bim_hbm, bim_ref), (wg_hbm, wg_ref), (wu_hbm, wu_ref),
             (cre_hbm, cre_ref), (cim_hbm, cim_ref), (wd_hbm, wd_ref)])]

        def wait_w(*ks):
            @pl.when(step == 0)
            def _():
                for k in ks:
                    copies[k].wait()

        @pl.when(step == 0)
        def _init():
            for cp in copies:
                cp.start()
            lre = lre_ref[...].astype(jnp.float32).reshape(1, P)
            lim = lim_ref[...].astype(jnp.float32).reshape(1, P)
            ldt = ldt_ref[...].astype(jnp.float32).reshape(1, P)
            dt = jnp.exp(ldt).astype(jnp.bfloat16).astype(jnp.float32)
            ar = dt * lre
            ai = dt * lim
            mag = jnp.exp(ar)
            lbr = mag * jnp.cos(ai)
            lbi = mag * jnp.sin(ai)
            nr = lbr - 1.0
            ni = lbi
            den = lre * lre + lim * lim
            cr = (nr * lre + ni * lim) / den
            ci = (ni * lre - nr * lim) / den
            par_ref[0:8, :] = jnp.broadcast_to(lbr, (8, P))
            par_ref[8:16, :] = jnp.broadcast_to(-lbi, (8, P))
            par_ref[16:24, :] = jnp.broadcast_to(2.0 * cr, (8, P))
            par_ref[24:32, :] = jnp.broadcast_to(2.0 * ci, (8, P))
            par_ref[32:40, :] = jnp.broadcast_to(dsk_ref[...].astype(jnp.float32).reshape(1, D), (8, D))
            k = (lax.broadcasted_iota(jnp.int32, (CH, P), 0) + 1).astype(jnp.float32)
            m = jnp.exp(k * ar)
            th = k * ai
            tr = m * jnp.cos(th)
            ti = -(m * jnp.sin(th))
            for i in range(CH):
                pwr_ref[8 * i:8 * i + 8, :] = jnp.broadcast_to(tr[i:i + 1, :], (8, P))
                pwi_ref[8 * i:8 * i + 8, :] = jnp.broadcast_to(ti[i:i + 1, :], (8, P))
            car_ref[...] = jnp.zeros_like(car_ref)

        xb = x_ref[...]
        xf = xb.astype(jnp.float32)
        mean = jnp.mean(xf, axis=-1, keepdims=True)
        cen = xf - mean
        var = jnp.mean(cen * cen, axis=-1, keepdims=True)
        m_b = mean.astype(jnp.bfloat16)
        v_b = var.astype(jnp.bfloat16)
        num = (xb - m_b)
        den = jnp.sqrt(v_b + jnp.asarray(1e-5, jnp.bfloat16))
        xn = (num.astype(jnp.float32) / den.astype(jnp.float32)).astype(jnp.bfloat16).astype(jnp.float32)
        for j in range(8):
            for c in range(ND):
                xs_ref[c, j * PITCH:j * PITCH + CH, :] = xn[j * CH:(j + 1) * CH, c * 128:(c + 1) * 128]

        for i2 in range(CH // 2):
            for c in range(ND):
                a = xs_ref[c, pl.ds(2 * i2, 8, stride=PITCH), :]
                b = xs_ref[c, pl.ds(2 * i2 + 1, 8, stride=PITCH), :]
                xp_ref[16 * i2:16 * i2 + 16, c * 128:(c + 1) * 128] = jnp.concatenate([a, b], axis=0).astype(jnp.bfloat16)
        xp = xp_ref[...]

        wait_w(0, 1)
        bur_ref[...] = lax.dot_general(xp, bre_ref[...], _NT, preferred_element_type=jnp.float32)
        bui_ref[...] = lax.dot_general(xp, bim_ref[...], _NT, preferred_element_type=jnp.float32)

        lbr = par_ref[0:8, :]
        lbi = par_ref[8:16, :]
        cr = par_ref[16:24, :]
        ci = par_ref[24:32, :]

        def body(i, carry):
            hr, hi = carry
            r0 = i * 8 if isinstance(i, int) else pl.multiple_of(i * 8, 8)
            br = bur_ref[pl.ds(r0, 8), :]
            bi = bui_ref[pl.ds(r0, 8), :]
            ur = cr * br - ci * bi
            ui = cr * bi + ci * br
            r = lbr * hr - lbi * hi + ur
            im = lbr * hi + lbi * hr - ui
            bur_ref[pl.ds(r0, 8), :] = r
            bui_ref[pl.ds(r0, 8), :] = im
            return r, im

        z = jnp.zeros((8, P), jnp.float32)
        if UNROLL >= CH:
            fr, fi = z, z
            for i in range(CH):
                fr, fi = body(i, (fr, fi))
        else:
            fr, fi = lax.fori_loop(0, CH, body, (z, z), unroll=UNROLL)

        lcr = pwr_ref[TL - 1:TL, :]
        lci = pwi_ref[TL - 1:TL, :]
        c_r = car_ref[0:1, :]
        c_i = car_ref[1:2, :]
        rows_r, rows_i = [], []
        for j in range(8):
            rows_r.append(c_r)
            rows_i.append(c_i)
            f_r = fr[j:j + 1, :]
            f_i = fi[j:j + 1, :]
            n_r = lcr * c_r - lci * c_i + f_r
            n_i = lcr * c_i + lci * c_r + f_i
            c_r, c_i = n_r, n_i
        car_ref[0:1, :] = c_r
        car_ref[1:2, :] = c_i
        cvr = jnp.concatenate(rows_r, axis=0)
        cvi = jnp.concatenate(rows_i, axis=0)

        RB = 64
        for b in range(TL // RB):
            sl = slice(b * RB, (b + 1) * RB)
            pwr = pwr_ref[sl, :].reshape(RB // 8, 8, P)
            pwi = pwi_ref[sl, :].reshape(RB // 8, 8, P)
            hr = bur_ref[sl, :].reshape(RB // 8, 8, P) + (pwr * cvr[None] - pwi * cvi[None])
            hi = bui_ref[sl, :].reshape(RB // 8, 8, P) + (pwr * cvi[None] + pwi * cvr[None])
            hcat_ref[sl, 0:P] = hr.reshape(RB, P).astype(jnp.bfloat16)
            hcat_ref[sl, P:2 * P] = hi.reshape(RB, P).astype(jnp.bfloat16)

        wait_w(4, 5)
        y = lax.dot_general(hcat_ref[:, 0:P], cre_ref[...], _NT, preferred_element_type=jnp.float32)
        y = y + lax.dot_general(hcat_ref[:, P:2 * P], cim_ref[...], _NT, preferred_element_type=jnp.float32)
        dsk = par_ref[32:33, :].astype(jnp.bfloat16)
        skip = (xp * dsk).astype(jnp.float32)

        wait_w(2, 3, 6)
        g = lax.dot_general(xp, wg_ref[...], _NT, preferred_element_type=jnp.float32).astype(jnp.bfloat16).astype(jnp.float32)
        u = lax.dot_general(xp, wu_ref[...], _NT, preferred_element_type=jnp.float32).astype(jnp.bfloat16).astype(jnp.float32)
        a = (_gelu_tanh(g).astype(jnp.bfloat16).astype(jnp.float32) * u).astype(jnp.bfloat16)
        ffn = jnp.dot(a, wd_ref[...], preferred_element_type=jnp.float32).astype(jnp.bfloat16).astype(jnp.float32)

        tot = (y + skip) + ffn
        for c in range(ND):
            ys_ref[c] = tot[:, c * 128:(c + 1) * 128]

        for j in range(8):
            for mblk in range(CH // 8):
                r0 = j * CH + mblk * 8
                for c in range(ND):
                    v = ys_ref[c, pl.ds(64 * mblk + j, 8, stride=8), :]
                    o_ref[r0:r0 + 8, c * 128:(c + 1) * 128] = xf[r0:r0 + 8, c * 128:(c + 1) * 128] + v

    return kernel, CH, PITCH


@functools.partial(jax.jit, static_argnames=("TL", "UNROLL"))
def pallas_parallel_sum__ssm_conv_s5__geglu_ffn__prompt_kernel(
    A_x, A_Lambda_re, A_Lambda_im, A_B_re, A_B_im, A_C_re, A_C_im, A_log_dt, A_Dskip,
    B_x, B_w_gate, B_w_up, B_w_down, TL=512, UNROLL=64):
    Bsz, L, D = A_x.shape
    P = A_Lambda_re.shape[0]
    F = B_w_gate.shape[1]
    assert Bsz == 1 and L % TL == 0
    x2 = A_x.reshape(L, D)
    kernel, CH, PITCH = _make_kernel(TL, D, P, F, UNROLL)
    full = lambda shp: pl.BlockSpec(shp, lambda i: (0,) * len(shp))
    out = pl.pallas_call(
        kernel,
        grid=(L // TL,),
        in_specs=[
            pl.BlockSpec((TL, D), lambda i: (i, 0)),
            full((P,)), full((P,)), full((P,)), full((D,)),
        ] + [pl.BlockSpec(memory_space=pl.ANY)] * 7,
        out_specs=pl.BlockSpec((TL, D), lambda i: (i, 0)),
        out_shape=jax.ShapeDtypeStruct((L, D), jnp.float32),
        scratch_shapes=[
            pltpu.VMEM((P, D), jnp.bfloat16), pltpu.VMEM((P, D), jnp.bfloat16),
            pltpu.VMEM((D, P), jnp.bfloat16), pltpu.VMEM((D, P), jnp.bfloat16),
            pltpu.VMEM((F, D), jnp.bfloat16), pltpu.VMEM((F, D), jnp.bfloat16), pltpu.VMEM((F, D), jnp.bfloat16),
            pltpu.SemaphoreType.DMA((7,)),
            pltpu.VMEM((40, P), jnp.float32),
            pltpu.VMEM((TL, P), jnp.float32),
            pltpu.VMEM((TL, P), jnp.float32),
            pltpu.VMEM((8, P), jnp.float32),
            pltpu.VMEM((D // 128, 8 * PITCH, 128), jnp.float32),
            pltpu.VMEM((TL, D), jnp.bfloat16),
            pltpu.VMEM((TL, P), jnp.float32),
            pltpu.VMEM((TL, P), jnp.float32),
            pltpu.VMEM((TL, 2 * P), jnp.bfloat16),
            pltpu.VMEM((D // 128, TL, 128), jnp.float32),
        ],
        compiler_params=pltpu.CompilerParams(
            dimension_semantics=("arbitrary",),
            vmem_limit_bytes=100 * 1024 * 1024,
        ),
    )(x2, A_Lambda_re, A_Lambda_im, A_log_dt, A_Dskip,
      A_B_re, A_B_im, A_C_re, A_C_im, B_w_gate.T, B_w_up.T, B_w_down)
    return out.reshape(Bsz, L, D)
```

```python
import functools
import math
import jax
import jax.numpy as jnp
from jax import lax
import jax.experimental.pallas as pl
import jax.experimental.pallas.tpu as pltpu

_NT = (((1,), (1,)), ((), ()))


def _gelu_tanh(x):
    c = math.sqrt(2.0 / math.pi)
    return 0.5 * x * (1.0 + jnp.tanh(c * (x + 0.044715 * (x * x * x))))


def _make_kernel(T, TL, D, P, F):
    CH = TL // 8
    PITCH = CH + 8
    ND = D // 128
    GUC = [(128 * k, 128) for k in range(10)] + [(1280, F - 1280)]

    def kernel(x_hbm, lre_ref, lim_ref, ldt_ref, dsk_ref, bre_hbm, bim_hbm, cre_hbm, cim_hbm,
               wg_hbm, wu_hbm, wd_hbm, o_hbm,
               x_ref, bre_ref, bim_ref, cre_ref, cim_ref, wg_ref, wu_ref, wd_ref, wsem, xsem, osem,
               par_ref, pwr_ref, pwi_ref, car_ref, xs_ref, xp_ref, xq_ref, bur_ref, bui_ref, hcat_ref,
               a_ref, ys_ref, fin_ref, ob_ref):
        step = pl.program_id(0)

        wcp = [pltpu.make_async_copy(h, v, wsem.at[k]) for k, (h, v) in enumerate(
            [(bre_hbm, bre_ref), (bim_hbm, bim_ref), (wg_hbm, wg_ref), (wu_hbm, wu_ref),
             (wd_hbm, wd_ref), (cre_hbm, cre_ref), (cim_hbm, cim_ref)])]

        def xcp(t):
            r = t * TL if isinstance(t, int) else pl.multiple_of(t * TL, TL)
            return pltpu.make_async_copy(x_hbm.at[pl.ds(r, TL)], x_ref.at[pl.ds(r, TL)], xsem.at[t])

        def ocp(t, j):
            r = pl.multiple_of(t * TL + j * CH, CH)
            return pltpu.make_async_copy(ob_ref.at[pl.ds(j * CH, CH)], o_hbm.at[pl.ds(r, CH)], osem.at[j])

        def ocp_col(t, c):
            r = pl.multiple_of(t * TL, TL)
            return pltpu.make_async_copy(ob_ref.at[:, pl.ds(c * 128, 128)],
                                         o_hbm.at[pl.ds(r, TL), pl.ds(c * 128, 128)], osem.at[c])

        NQ = 8
        QI = CH // NQ
        QR = 8 * QI

        def ln_permute_piece(tile, q):
            for j in range(8):
                src = pl.multiple_of(tile * TL + j * CH + q * QI, QI)
                xb = x_ref[pl.ds(src, QI), :]
                xf = xb.astype(jnp.float32)
                mean = jnp.mean(xf, axis=-1, keepdims=True)
                cen = xf - mean
                var = jnp.mean(cen * cen, axis=-1, keepdims=True)
                m_b = mean.astype(jnp.bfloat16)
                v_b = var.astype(jnp.bfloat16)
                num = (xb - m_b)
                den = jnp.sqrt(v_b + jnp.asarray(1e-5, jnp.bfloat16))
                xn = (num.astype(jnp.float32) / den.astype(jnp.float32)).astype(jnp.bfloat16).astype(jnp.float32)
                r0 = j * PITCH + q * QI
                for c in range(ND):
                    xs_ref[c, r0:r0 + QI, :] = xn[:, c * 128:(c + 1) * 128]
            for i2 in range(q * QI // 2, (q + 1) * QI // 2):
                for c in range(ND):
                    a = xs_ref[c, pl.ds(2 * i2, 8, stride=PITCH), :]
                    b = xs_ref[c, pl.ds(2 * i2 + 1, 8, stride=PITCH), :]
                    xq_ref[16 * i2:16 * i2 + 16, c * 128:(c + 1) * 128] = (
                        jnp.concatenate([a, b], axis=0).astype(jnp.bfloat16))

        def bproj_scan_piece(q, hr, hi):
            rs = slice(q * QR, (q + 1) * QR)
            xq = xq_ref[rs, :]
            bur_ref[rs, :] = lax.dot_general(xq, bre_ref[...], _NT, preferred_element_type=jnp.float32)
            bui_ref[rs, :] = lax.dot_general(xq, bim_ref[...], _NT, preferred_element_type=jnp.float32)
            lbr = par_ref[0:8, :]
            lbi = par_ref[8:16, :]
            cr = par_ref[16:24, :]
            ci = par_ref[24:32, :]
            for i in range(q * QI, (q + 1) * QI):
                r0 = i * 8
                br = bur_ref[r0:r0 + 8, :]
                bi = bui_ref[r0:r0 + 8, :]
                ur = cr * br - ci * bi
                ui = cr * bi + ci * br
                r = lbr * hr - lbi * hi + ur
                im = lbr * hi + lbi * hr - ui
                bur_ref[r0:r0 + 8, :] = r
                bui_ref[r0:r0 + 8, :] = im
                hr, hi = r, im
            if q == NQ - 1:
                fin_ref[0:8, :] = hr
                fin_ref[8:16, :] = hi
            return hr, hi

        @pl.when(step == 0)
        def _init():
            xcp(0).start()
            lre = lre_ref[...].astype(jnp.float32).reshape(1, P)
            lim = lim_ref[...].astype(jnp.float32).reshape(1, P)
            ldt = ldt_ref[...].astype(jnp.float32).reshape(1, P)
            dt = jnp.exp(ldt).astype(jnp.bfloat16).astype(jnp.float32)
            ar = dt * lre
            ai = dt * lim
            mag = jnp.exp(ar)
            lbr = mag * jnp.cos(ai)
            lbi = mag * jnp.sin(ai)
            nr = lbr - 1.0
            ni = lbi
            sc = jnp.maximum(jnp.abs(lre), jnp.abs(lim))
            qa = lre / sc
            qb = lim / sc
            den = (qa * qa + qb * qb) * sc
            cr = (nr * qa + ni * qb) / den
            ci = (ni * qa - nr * qb) / den
            l8r = jnp.broadcast_to(lbr, (8, P))
            l8i = jnp.broadcast_to(-lbi, (8, P))
            par_ref[0:8, :] = l8r
            par_ref[8:16, :] = l8i
            par_ref[16:24, :] = jnp.broadcast_to(2.0 * cr, (8, P))
            par_ref[24:32, :] = jnp.broadcast_to(2.0 * ci, (8, P))
            par_ref[32:40, :] = jnp.broadcast_to(dsk_ref[...].astype(jnp.float32).reshape(1, D), (8, D))
            tr, ti = l8r, l8i
            for i in range(CH):
                pwr_ref[8 * i:8 * i + 8, :] = tr
                pwi_ref[8 * i:8 * i + 8, :] = ti
                if i + 1 < CH:
                    tr, ti = l8r * tr - l8i * ti, l8r * ti + l8i * tr
            car_ref[...] = jnp.zeros_like(car_ref)
            wcp[0].start()
            wcp[1].start()
            xcp(0).wait()
            wcp[2].start()
            wcp[3].start()
            for t in range(1, min(T, 2)):
                xcp(t).start()
            for q in range(NQ):
                ln_permute_piece(0, q)
            wcp[0].wait()
            wcp[1].wait()
            hr = hi = jnp.zeros((8, P), jnp.float32)
            for q in range(NQ):
                hr, hi = bproj_scan_piece(q, hr, hi)
            wcp[2].wait()
            wcp[3].wait()
            wcp[4].start()
            wcp[5].start()
            wcp[6].start()
            for t in range(2, T):
                xcp(t).start()

        @pl.when(step < T - 1)
        def _():
            xcp(step + 1).wait()

        def carry_chain():
            lcr = pwr_ref[TL - 1:TL, :]
            lci = pwi_ref[TL - 1:TL, :]
            c_r = car_ref[0:1, :]
            c_i = car_ref[1:2, :]
            rows_r, rows_i = [], []
            for j in range(8):
                rows_r.append(c_r)
                rows_i.append(c_i)
                n_r = lcr * c_r - lci * c_i + fin_ref[j:j + 1, :]
                n_i = lcr * c_i + lci * c_r + fin_ref[8 + j:9 + j, :]
                c_r, c_i = n_r, n_i
            car_ref[0:1, :] = c_r
            car_ref[1:2, :] = c_i
            return jnp.concatenate(rows_r, axis=0), jnp.concatenate(rows_i, axis=0)

        def fixup():
            cvr, cvi = carry_chain()
            RB = 64
            for b in range(TL // RB):
                sl = slice(b * RB, (b + 1) * RB)
                pwr = pwr_ref[sl, :].reshape(RB // 8, 8, P)
                pwi = pwi_ref[sl, :].reshape(RB // 8, 8, P)
                fr = bur_ref[sl, :].reshape(RB // 8, 8, P) + (pwr * cvr[None] - pwi * cvi[None])
                fi = bui_ref[sl, :].reshape(RB // 8, 8, P) + (pwr * cvi[None] + pwi * cvr[None])
                hcat_ref[sl, 0:P] = fr.reshape(RB, P).astype(jnp.bfloat16)
                hcat_ref[sl, P:2 * P] = fi.reshape(RB, P).astype(jnp.bfloat16)

        def body(with_next):
            xp_ref[...] = xq_ref[...]
            if with_next:
                fixup()
            xp = xp_ref[...]

            def gu(s0, n):
                g = lax.dot_general(xp, wg_ref[s0:s0 + n, :], _NT, preferred_element_type=jnp.float32).astype(jnp.bfloat16).astype(jnp.float32)
                u = lax.dot_general(xp, wu_ref[s0:s0 + n, :], _NT, preferred_element_type=jnp.float32).astype(jnp.bfloat16).astype(jnp.float32)
                a_ref[:, s0:s0 + n] = (_gelu_tanh(g).astype(jnp.bfloat16).astype(jnp.float32) * u).astype(jnp.bfloat16)

            hr = hi = jnp.zeros((8, P), jnp.float32)
            for k, (s0, n) in enumerate(GUC):
                gu(s0, n)
                if with_next and k < NQ:
                    ln_permute_piece(step + 1, k)
                    hr, hi = bproj_scan_piece(k, hr, hi)

            if T == 1 or with_next:
                @pl.when(step == 0)
                def _():
                    wcp[4].wait()
                    wcp[5].wait()
                    wcp[6].wait()

            if T > 1:
                @pl.when(step > 0)
                def _():
                    for j in range(8):
                        ocp(step - 1, j).wait()

            if not with_next:
                fixup()
            base = pl.multiple_of(step * TL, TL)
            dsk = par_ref[32:33, :].astype(jnp.bfloat16)
            for c in range(ND):
                cs = slice(c * 128, (c + 1) * 128)
                y = lax.dot_general(hcat_ref[:, 0:P], cre_ref[cs, :], _NT, preferred_element_type=jnp.float32)
                y = y + lax.dot_general(hcat_ref[:, P:2 * P], cim_ref[cs, :], _NT, preferred_element_type=jnp.float32)
                y = y + (xp_ref[:, cs] * dsk[:, cs]).astype(jnp.float32)
                ffn = jnp.dot(a_ref[...], wd_ref[:, cs], preferred_element_type=jnp.float32)
                ys_ref[c] = y + ffn.astype(jnp.bfloat16).astype(jnp.float32)
                for j in range(8):
                    for mblk in range(CH // 8):
                        r0 = j * CH + mblk * 8
                        xr = x_ref[pl.ds(base + r0, 8), cs].astype(jnp.float32)
                        v = ys_ref[c, pl.ds(64 * mblk + j, 8, stride=8), :]
                        ob_ref[r0:r0 + 8, cs] = xr + v
                if not with_next:
                    ocp_col(step, c).start()
            if with_next:
                for j in range(8):
                    ocp(step, j).start()
            else:
                for c in range(ND):
                    ocp_col(step, c).wait()

        if T > 1:
            @pl.when(step < T - 1)
            def _():
                body(True)

        @pl.when(step == T - 1)
        def _():
            body(False)

    return kernel, CH, PITCH


@functools.partial(jax.jit, static_argnames=("TL",))
def pallas_parallel_sum__ssm_conv_s5__geglu_ffn__prompt_kernel(
    A_x, A_Lambda_re, A_Lambda_im, A_B_re, A_B_im, A_C_re, A_C_im, A_log_dt, A_Dskip,
    B_x, B_w_gate, B_w_up, B_w_down, TL=512):
    Bsz, L, D = A_x.shape
    P = A_Lambda_re.shape[0]
    F = B_w_gate.shape[1]
    assert Bsz == 1 and L % TL == 0 and D == P and D % 128 == 0 and 1280 < F <= 1408
    T = L // TL
    x2 = A_x.reshape(L, D)
    kernel, CH, PITCH = _make_kernel(T, TL, D, P, F)
    full = lambda shp: pl.BlockSpec(shp, lambda i: (0,) * len(shp))
    anyspec = pl.BlockSpec(memory_space=pl.ANY)
    out = pl.pallas_call(
        kernel,
        grid=(T,),
        in_specs=[anyspec, full((P,)), full((P,)), full((P,)), full((D,))] + [anyspec] * 7,
        out_specs=anyspec,
        out_shape=jax.ShapeDtypeStruct((L, D), jnp.float32),
        scratch_shapes=[
            pltpu.VMEM((L, D), jnp.bfloat16),
            pltpu.VMEM((P, D), jnp.bfloat16), pltpu.VMEM((P, D), jnp.bfloat16),
            pltpu.VMEM((D, P), jnp.bfloat16), pltpu.VMEM((D, P), jnp.bfloat16),
            pltpu.VMEM((F, D), jnp.bfloat16), pltpu.VMEM((F, D), jnp.bfloat16), pltpu.VMEM((F, D), jnp.bfloat16),
            pltpu.SemaphoreType.DMA((7,)),
            pltpu.SemaphoreType.DMA((T,)),
            pltpu.SemaphoreType.DMA((8,)),
            pltpu.VMEM((40, P), jnp.float32),
            pltpu.VMEM((TL, P), jnp.float32),
            pltpu.VMEM((TL, P), jnp.float32),
            pltpu.VMEM((8, P), jnp.float32),
            pltpu.VMEM((D // 128, 8 * PITCH, 128), jnp.float32),
            pltpu.VMEM((TL, D), jnp.bfloat16),
            pltpu.VMEM((TL, D), jnp.bfloat16),
            pltpu.VMEM((TL, P), jnp.float32),
            pltpu.VMEM((TL, P), jnp.float32),
            pltpu.VMEM((TL, 2 * P), jnp.bfloat16),
            pltpu.VMEM((TL, F), jnp.bfloat16),
            pltpu.VMEM((D // 128, TL, 128), jnp.float32),
            pltpu.VMEM((16, P), jnp.float32),
            pltpu.VMEM((TL, D), jnp.float32),
        ],
        compiler_params=pltpu.CompilerParams(
            dimension_semantics=("arbitrary",),
            vmem_limit_bytes=100 * 1024 * 1024,
        ),
    )(x2, A_Lambda_re, A_Lambda_im, A_log_dt, A_Dskip,
      A_B_re, A_B_im, A_C_re, A_C_im, B_w_gate.T, B_w_up.T, B_w_down)
    return out.reshape(Bsz, L, D)
```
